```python
import jax
import jax.numpy as jnp

def _softmax(x, axis=-1):
    return jax.nn.softmax(x, axis=axis)
def _gelu(x):
    return jax.nn.gelu(x, approximate=True)
def _silu(x):
    return jax.nn.silu(x)
def _sigmoid(x):
    return jax.nn.sigmoid(x)
def _layernorm(x, axis=-1, eps=1e-5):
    m = jnp.mean(x, axis=axis, keepdims=True)
    v = jnp.var(x, axis=axis, keepdims=True)
    return (x - m) / jnp.sqrt(v + eps)
def _scatter_add(tgt, idx, src, axis=0):
    return tgt.at[idx].add(src)
def _segment_sum(src, seg, n):
    return jax.ops.segment_sum(src, seg, n)
class _Rng:
    def __init__(self, key):
        self._k = key
    def _next(self):
        self._k, sub = jax.random.split(self._k)
        return sub
    def normal(self, shape):
        return jax.random.normal(self._next(), shape, dtype=jnp.bfloat16)
    def randint(self, lo, hi, shape):
        return jax.random.randint(self._next(), shape, lo, hi, dtype=jnp.int32)
    def uniform(self, shape, lo=0.0, hi=1.0):
        return jax.random.uniform(self._next(), shape, jnp.bfloat16, lo, hi)
    def permutation(self, n):
        return jax.random.permutation(self._next(), n)


kernel_name = 'standalone__gqa_block_cached__near_ridge'

def _fwd_setup_inputs():
    _rng = _Rng(jax.random.key(int.from_bytes(__import__("os").urandom(4), "little")))
    _w = (lambda a: (lambda t: t.astype(jnp.bfloat16) if jnp.issubdtype(t.dtype, jnp.floating) else t)(jnp.asarray(a)))
    B, Sq, D = 16, 64, 640
    Hq, Hkv, Sk, Dh = 32, 32, 512, 192
    assert Hq % Hkv == 0, (Hq, Hkv)
    return {
        "x": _w((lambda *s: _rng.normal(s) * 0.05)(B, Sq, D)),
        "k_cache": _w((lambda *s: _rng.normal(s) * 0.05)(B, Hkv, Sk, Dh)),
        "v_cache": _w((lambda *s: _rng.normal(s) * 0.05)(B, Hkv, Sk, Dh)),
        "wq": _w((lambda *s: _rng.normal(s) * 0.05)(D, Hq * Dh) * (D ** -0.5)),
        "wo": _w((lambda *s: _rng.normal(s) * 0.05)(Hq * Dh, D) * ((Hq * Dh) ** -0.5)),
    }

def _fwd_reference(x, k_cache, v_cache, wq, wo):
    B, Sq, D = x.shape
    Hq, Dh = 32, 192
    Hkv = k_cache.shape[1]
    rep = Hq // Hkv
    q = (lambda x, *d: x.transpose(*d))((x @ wq).reshape(B, Sq, Hq, Dh), 0, 2, 1, 3)
    k = jnp.repeat(k_cache, rep, axis=1)
    v = jnp.repeat(v_cache, rep, axis=1)
    scores = jnp.einsum("bhqd,bhkd->bhqk", q, k) * (Dh ** -0.5)
    p = _softmax(scores, axis=-1)
    o = jnp.einsum("bhqk,bhkd->bhqd", p, v)
    return (lambda x, *d: x.transpose(*d))(o, 0, 2, 1, 3).reshape(B, Sq, Hq * Dh) @ wo


def setup_inputs():
    _inp = _fwd_setup_inputs()
    _gk = jax.random.fold_in(jax.random.key(int.from_bytes(__import__("os").urandom(4), "little")), 2**31 - 1)
    _shapes = [[16, 64, 640]]
    _dtypes = ['bfloat16']
    _gks = jax.random.split(_gk, len(_shapes))
    _gs = [jax.random.normal(k, s, dtype=jnp.dtype(d)) * 0.05 for k, s, d in zip(_gks, _shapes, _dtypes)]
    _inp["grad_out"] = _gs[0]
    return _inp

def reference(x, k_cache, v_cache, wq, wo, grad_out):
    _const = dict()
    def _f(*_d):
        return _fwd_reference(**{'x': _d[0], 'k_cache': _d[1], 'v_cache': _d[2], 'wq': _d[3], 'wo': _d[4], **_const})
    _out, _vjp = jax.vjp(_f, x, k_cache, v_cache, wq, wo)
    _grads = _vjp(grad_out)
    _out0 = jnp.asarray(_out)
    return (_out0, *[jnp.asarray(_g) for _g in _grads])
```

```python
import jax
import jax.numpy as jnp
from jax import lax
import jax.experimental.pallas as pl
import jax.experimental.pallas.tpu as pltpu

F32 = jnp.float32
BF16 = jnp.bfloat16
LOG2E = 1.4426950408889634

RING = 15
W_RING, DW_RING = 6, 5
BLOCK = 4
READ_ROWS = (8,) * 12
WRITE_ROWS = (40,) * 8 + (32, 32)
POINTS = 5
READ_PHASES = ((1, 6), (4, 9), (5, 12), (10, 103), (227, 181), (425, 256))
SPARE_POINT, SPARE_STEPS = 1, (5, 6, 18, 46, 52, 62, 85, 86, 93, 100, 102)
WRITE_PHASES = ((24, 20), (64, 40), (102, 61), (124, 62))
SYNC_STEP, SYNC_UNIT = 84, 38
EARLY_ROWS = 5


def _nn(a, b):
    return lax.dot_general(a, b, (((1,), (0,)), ((), ())), preferred_element_type=F32)


def _nt(a, b):
    return lax.dot_general(a, b, (((1,), (1,)), ((), ())), preferred_element_type=F32)


def _stack(parts):
    return jnp.concatenate(parts, axis=0).astype(BF16)


def _low_lanes(shape):
    return lax.broadcasted_iota(jnp.int32, shape, 1) < 64


def _scores(a, m_t):
    t = a[:, 128:256]
    low = _low_lanes(t.shape)
    first = _nn(a[:, 0:128].astype(BF16), m_t[0:128, :])
    mid = _nn(_stack([jnp.where(low, t, 0.0), jnp.where(low, 0.0, t)]), m_t[128:256, :])
    last = _nn(a[:, 256:384].astype(BF16), m_t[256:384, :])
    return first + mid[0:64], last + mid[64:128]


def _apply(w, m_t):
    first = _nt(w[0].astype(BF16), m_t[0:128, :])
    mid = _nt(_stack(w), m_t[128:256, :])
    last = _nt(w[1].astype(BF16), m_t[256:384, :])
    return jnp.concatenate(
        [first, jnp.where(_low_lanes(first.shape), mid[0:64], mid[64:128]), last], axis=1)


def _softmax(s):
    e = jnp.exp2((s - jnp.max(s, axis=1, keepdims=True)) * LOG2E)
    total = jnp.sum(e, axis=1, keepdims=True)
    r = pl.reciprocal(total, approx=True)
    return e * (r * (2.0 - total * r))


def _softmax_grad(p, dp):
    return [a * (b - jnp.sum(a * b, axis=1, keepdims=True)) for a, b in zip(p, dp)]


def _cache_grad(a, w0, w1, dst):
    a_t = a.astype(BF16).T
    dh = a_t.shape[0] // 2
    for h in range(2):
        u = pltpu.bitcast(a_t[h * dh:(h + 1) * dh], jnp.uint32)
        low, zero = _low_lanes(u.shape), jnp.zeros_like(u)
        lhs = jnp.concatenate([pltpu.bitcast(jnp.where(low, u, zero), BF16),
                               pltpu.bitcast(jnp.where(low, zero, u), BF16)], axis=0)
        r = _nn(lhs, _stack([w0[h], w1[h]])).astype(BF16)
        dst[0, h * dh:(h + 1) * dh, :] = r[:dh]
        dst[1, h * dh:(h + 1) * dh, :] = r[dh:]


def _spread(a, b):
    keys = [((i // 2 + 0.5) / len(part), which, i)
            for which, part in enumerate((a, b)) for i in range(len(part))]
    return [(a, b)[which][i] for _, which, i in sorted(keys)]


def _mod(v, n):
    return v - n * lax.shift_right_logical(v * (65536 // n + 1), 16)


def _lookup(k, table):
    value = 0
    for key, v in table:
        value = jnp.where(k >= key, v, value)
    return value


@jax.jit
def pallas_standalone__gqa_block_cached__near_ridge_kernel(
    x: jax.Array,
    k_cache: jax.Array,
    v_cache: jax.Array,
    wq: jax.Array,
    wo: jax.Array,
    grad_out: jax.Array,
):
    nb, sq, d = x.shape
    _, nh, sk, dh = k_cache.shape
    assert (nb, sq, d, nh, dh) == (16, 64, 640, 32, 192) and wq.shape == (d, nh * dh)
    pw = 2 * dh
    n_pairs = nh // 2
    pair_steps = nb // 2
    n_steps = n_pairs * pair_steps
    n_units = n_steps // 2
    scale = dh ** -0.5
    spare_words = [(w, sum(1 << (s - w) for s in SPARE_STEPS if w <= s < w + 16))
                   for w in range(0, n_steps, 16)]

    def kernel(x_hbm, k_hbm, v_hbm, wq_hbm, wo_hbm, g_hbm,
               out_hbm, dx_hbm, dk_hbm, dv_hbm, dwq_hbm, dwo_hbm,
               x_v, g_v, wq_v, wo_v, k_v, v_v, dk_v, dv_v,
               out_acc, dx_acc, out_v, dx_v, dwq_acc, dwo_acc, dwq_v, dwo_v, sems):
        caches, cache_grads = ((k_hbm, k_v), (v_hbm, v_v)), ((dk_hbm, dk_v), (dv_hbm, dv_v))
        weights, weight_grads = (wq_hbm, wq_v, wo_hbm, wo_v), (dwq_hbm, dwq_v, dwo_hbm, dwo_v)
        inputs, outputs = ((x_hbm, x_v), (g_hbm, g_v)), ((out_hbm, out_v), (dx_hbm, dx_v))
        sem_weights, sem_first, sem_second, sem_last = (sems.at[2 * RING + i] for i in range(4))

        def weight_part(refs, p, slot, part, parts, pieces):
            q_hbm, q_v, o_hbm, o_v = refs
            a, b = d // parts, pw // parts
            q_rows = pl.ds(pl.multiple_of(part * a, 8), a)
            o_row = pl.multiple_of(part * b, 8)
            views = ((q_hbm.at[q_rows, pl.ds(pl.multiple_of(p * pw, pw), pw)],
                      q_v.at[slot, q_rows], a // pieces),
                     (o_hbm.at[pl.ds(pl.multiple_of(p * pw + o_row, 8), b), :],
                      o_v.at[slot, pl.ds(o_row, b)], b // pieces))
            return [(h.at[pl.ds(i * n, n)], v.at[pl.ds(i * n, n)], queue)
                    for i in range(pieces) for queue, (h, v, n) in enumerate(views)]

        def cache_part(refs, p, batch, slot, first, count, rows, row0=0):
            size = sum(rows)
            in_unit = pl.ds(row0 if size == pw else pl.multiple_of(row0, 8), size)
            views = [(h.at[pl.ds(batch, count), pl.ds(pl.multiple_of(p * pw + row0, 8), size), :],
                      v.at[slot, pl.ds(first, count), in_unit, :]) for h, v in refs]
            pieces = [pl.ds(sum(rows[:i]), n) for i, n in enumerate(rows)]
            return [(h.at[:, r, :], v.at[:, r, :], queue)
                    for r in pieces for queue, (h, v) in enumerate(views)]

        def row_part(refs, j, rows):
            return [(h.at[j, pl.ds(r, rows)], v.at[j, pl.ds(r, rows)], queue)
                    for r in range(0, 2 * sq, rows) for queue, (h, v) in enumerate(refs)]

        def outgoing(copies):
            return [(v, h, 0) for h, v, _ in copies]

        def read_group(c):
            m, p, e = lax.shift_right_logical(c, 2), lax.shift_right_logical(c, 4), c & 15
            nxt = jnp.minimum(p + 1, n_pairs - 1)
            rows = (lax.shift_right_logical(e, 1), pl.ds(pl.multiple_of((e & 1) * sq, sq), sq))
            cache = cache_part(caches, p, 4 * (m & 3), _mod(m, RING), 0, 4, READ_ROWS,
                               (c & 3) * (pw // 4))
            return cache, [
                (p < n_pairs - 1, weight_part(weights, nxt, _mod(nxt, W_RING), e, 16, 1)),
                (p == 0, [(h.at[rows], v.at[rows], queue) for queue, (h, v) in enumerate(inputs)])]

        def write_unit(m):
            p = lax.shift_right_logical(m, 2)
            src = jnp.minimum(p, n_pairs - 2)
            cache = cache_part(cache_grads, p, 4 * (m & 3), _mod(m, RING), 0, 4, WRITE_ROWS)
            return (outgoing(cache[0::2] + cache[1::2]), p != n_pairs - 2,
                    outgoing(weight_part(weight_grads, src, _mod(src, DW_RING), m & 3, 4, 2)))

        def first_weights():
            return sum([weight_part(weights, 0, 0, u, 4, 4) for u in range(4)], [])

        def first_reads(j):
            copies = row_part(inputs, j, 32) + cache_part(caches, 0, 2 * j, 0, 2 * j, 2, (24,) * 16)
            return copies + (weight_part(weights, 1, 1, 0, 4, 4) if j else [])

        def early_writes():
            js = pl.ds(0, EARLY_ROWS)
            return [(v.at[js, pl.ds(r, 32)], h.at[js, pl.ds(r, 32)], 0)
                    for r in range(0, 2 * sq, 32) for h, v in outputs]

        def last_writes(stage):
            p, slot = n_pairs - 1, (n_units - 1) % RING
            if stage == 0:
                rows = [row_part(outputs, j, 64) for j in range(EARLY_ROWS, pair_steps - 1)]
                return outgoing(_spread(
                    cache_part(cache_grads, p, nb - 4, slot, 0, 2, WRITE_ROWS),
                    sum(rows, []) + weight_part(weight_grads, p - 1, (p - 1) % DW_RING, 3, 4, 2)))
            if stage in (1, 4):
                cache = cache_part(cache_grads, p, nb - 2, slot, 2, 2, WRITE_ROWS)
                return outgoing(cache[1::2] if stage == 1 else cache[0::2])
            rows = row_part(outputs, pair_steps - 1, 64)
            dw = sum([weight_part(weight_grads, p, p % DW_RING, u, 4, 2) for u in range(4)], [])
            return outgoing(_spread(dw[1::2], rows[0::2]) if stage == 2
                            else _spread(dw[0::2], rows[1::2]))

        def start(copies, sem):
            for src, dst, queue in copies:
                pltpu.make_async_copy(src, dst, sem).start(priority=queue)

        def wait(copies, sem):
            for src, dst, _ in copies:
                pltpu.make_async_copy(src, dst, sem).wait()

        def wait_written(m):
            cache, has_dw, dw = write_unit(m)
            sem = sems.at[RING + _mod(m, RING)]
            wait(cache, sem)
            pl.when(has_dw)(lambda: wait(dw, sem))

        def acquire(m):
            groups = [read_group(4 * m + q) for q in range(4)]
            sem = sems.at[_mod(m, RING)]
            wait(sum([cache for cache, _ in groups], []), sem)
            for n in range(2):
                pl.when(groups[0][1][n][0])(
                    lambda: wait(sum([more[n][1] for _, more in groups], []), sem))
            pl.when((m >= RING) & (m - RING != SYNC_UNIT))(lambda: wait_written(m - RING))

        def transfers(i, n_read, n_written, final):
            on = n_written < _lookup(i, WRITE_PHASES)
            cache, has_dw, dw = write_unit(n_written)
            sem, dw_on = sems.at[RING + _mod(n_written, RING)], on & has_dw
            todo = {"write": _spread([(on, c, sem) for c in cache], [(dw_on, c, sem) for c in dw]),
                    "more": []}
            n_written = n_written + jnp.where(on, 1, 0)
            for point in range(POINTS):
                on = n_read < _lookup(POINTS * i + point, READ_PHASES)
                if point == SPARE_POINT:
                    on = on & ((lax.shift_right_logical(_lookup(i, spare_words), i & 15) & 1) == 1)
                group = jnp.minimum(n_read, 4 * n_units - 1)
                cache, more = read_group(group)
                sem = sems.at[_mod(lax.shift_right_logical(group, 2), RING)]
                todo[point] = [(on, c, sem) for c in cache]
                for cond, copies in more:
                    both = on & cond
                    todo["more"] += [(both, c, sem) for c in copies]
                n_read = n_read + jnp.where(on, 1, 0)
            if final:
                for stage in (1, 2, 3):
                    todo["last", stage] = [(i == n_steps - 1, c, sem_last)
                                           for c in last_writes(stage)]
            return todo, (n_read, n_written)

        def compute(i, send, may_begin, may_end):
            p, j, m = lax.shift_right_logical(i, 3), i & 7, lax.shift_right_logical(i, 1)
            at = (_mod(m, RING), pl.ds(2 * (i & 1), 2))
            k_t, v_t, dk_t, dv_t = k_v.at[at], v_v.at[at], dk_v.at[at], dv_v.at[at]
            wq_p, wo_p = wq_v.at[_mod(p, W_RING)], wo_v.at[_mod(p, W_RING)]

            def add_weight_grad(acc, staged, a, b):
                term = _nn(a.T, b)
                total = (jnp.where(j == 0, 0.0, acc[...]) if may_begin else acc[...]) + term
                acc[...] = total
                if may_end:
                    staged[_mod(p, DW_RING)] = total.astype(BF16)

            send(0)
            q = _nn(x_v[j], wq_p[...]) * scale
            s0 = _scores(q[:sq], k_t.at[0])
            send(1)
            do = _nt(g_v[j], wo_p[...])
            send("more")
            s1 = _scores(q[sq:], k_t.at[1])
            p0 = [_softmax(t) for t in s0]
            o0 = _apply(p0, v_t.at[0])
            dp0 = _scores(do[:sq], v_t.at[0])
            p1 = [_softmax(t) for t in s1]
            o1 = _apply(p1, v_t.at[1])
            send(2)
            _cache_grad(do, p0, p1, dv_t)
            dp1 = _scores(do[sq:], v_t.at[1])
            ds0 = _softmax_grad(p0, dp0)
            send("write")
            send(("last", 1))
            dq0 = _apply(ds0, k_t.at[0]) * scale
            ds1 = _softmax_grad(p1, dp1)
            o = _stack([o0, o1])
            add_weight_grad(dwo_acc, dwo_v, o, g_v[j])
            send(3)
            dq1 = _apply(ds1, k_t.at[1]) * scale
            send(4)
            total = out_acc[j] + _nn(o, wo_p[...])
            out_acc[j] = total
            out_v[j] = total.astype(BF16)
            send(("last", 2))
            dq = _stack([dq0, dq1])
            add_weight_grad(dwq_acc, dwq_v, x_v[j], dq)
            total = dx_acc[j] + _nt(dq, wq_p[...])
            dx_acc[j] = total
            dx_v[j] = total.astype(BF16)
            send(("last", 3))
            _cache_grad(q, ds0, ds1, dk_t)

        def step(i, counts, may_begin=True, may_end=True, final=True):
            todo, counts = transfers(i, *counts, final)

            def send(point):
                for n, (cond, copy, sem) in enumerate(todo.get(point, [])):
                    pl.when(cond & (i >= 0) if n & 2 else cond)(lambda: start([copy], sem))

            compute(i, send, may_begin, may_end)
            return counts

        def single_step(i, counts):
            pl.when(i == 1)(lambda: wait(first_reads(1), sem_second))
            pl.when((i > 1) & ((i & 1) == 0))(lambda: acquire(lax.shift_right_logical(i, 1)))
            pl.when(i == n_steps - 3)(lambda: start(early_writes(), sem_last))

            @pl.when(i == n_steps - 2)
            def _():
                cache, _, dw = write_unit(n_units - 2)
                start(_spread(cache, dw), sems.at[RING + (n_units - 2) % RING])

            pl.when(i == n_steps - 1)(lambda: start(last_writes(0), sem_last))
            return step(i, counts)

        def block(b, counts):
            i = BLOCK * (b + 1)
            pl.when(i == SYNC_STEP)(lambda: wait_written(SYNC_UNIT))
            for u in range(0, BLOCK, 2):
                acquire(lax.shift_right_logical(i + u, 1))
            for u in range(BLOCK):
                counts = step(i + u, counts, u == 0, u == BLOCK - 1, False)
            return counts

        def half(h, counts):
            begin = h * (n_steps - BLOCK)
            counts = lax.fori_loop(begin, begin + BLOCK, single_step, counts)
            return lax.fori_loop(0, (1 - h) * (n_steps // BLOCK - 2), block, counts)

        def zero(j, carry):
            out_acc[j] = jnp.zeros(out_acc.shape[1:], F32)
            dx_acc[j] = jnp.zeros(dx_acc.shape[1:], F32)
            for acc in (dwq_acc, dwo_acc):
                n = acc.shape[0] // pair_steps
                acc[pl.ds(pl.multiple_of(j * n, 8), n), :] = jnp.zeros((n, acc.shape[1]), F32)
            return carry

        start(first_weights(), sem_weights)
        start(first_reads(0), sem_first)
        lax.fori_loop(0, pair_steps, zero, None)
        wait(first_weights(), sem_weights)
        start(first_reads(1)[:12], sem_second)
        wait(first_reads(0), sem_first)
        start(first_reads(1)[12:], sem_second)
        lax.fori_loop(0, 2, half, (4, 0))
        start(last_writes(4), sem_last)

        def drain(m, carry):
            wait_written(m)
            return carry

        lax.fori_loop(n_units - RING, n_units - 1, drain, None)
        wait(early_writes() + sum([last_writes(stage) for stage in range(5)], []), sem_last)

    def transposed(c):
        return jnp.swapaxes(c, 2, 3).reshape(nb, nh * dh, sk)

    def restored(c):
        return jnp.swapaxes(c.reshape(nb, nh, dh, sk), 2, 3)

    rows = (pair_steps, 2 * sq, d)
    hbm = pl.BlockSpec(memory_space=pl.ANY)
    vmem = pltpu.VMEM
    out, dx, dk, dv, dwq, dwo = pl.pallas_call(
        kernel,
        in_specs=[hbm] * 6,
        out_specs=[hbm] * 6,
        out_shape=[
            jax.ShapeDtypeStruct(rows, x.dtype),
            jax.ShapeDtypeStruct(rows, x.dtype),
            jax.ShapeDtypeStruct((nb, nh * dh, sk), k_cache.dtype),
            jax.ShapeDtypeStruct((nb, nh * dh, sk), v_cache.dtype),
            jax.ShapeDtypeStruct(wq.shape, wq.dtype),
            jax.ShapeDtypeStruct(wo.shape, wo.dtype),
        ],
        scratch_shapes=[
            vmem(rows, BF16), vmem(rows, BF16),
            vmem((W_RING, d, pw), BF16), vmem((W_RING, pw, d), BF16),
            vmem((RING, 4, pw, sk), BF16), vmem((RING, 4, pw, sk), BF16),
            vmem((RING, 4, pw, sk), BF16), vmem((RING, 4, pw, sk), BF16),
            vmem(rows, F32), vmem(rows, F32), vmem(rows, BF16), vmem(rows, BF16),
            vmem((d, pw), F32), vmem((pw, d), F32),
            vmem((DW_RING, d, pw), BF16), vmem((DW_RING, pw, d), BF16),
            pltpu.SemaphoreType.DMA((2 * RING + 4,)),
        ],
        compiler_params=pltpu.CompilerParams(
            vmem_limit_bytes=120 * 1024 * 1024, disable_bounds_checks=True),
        name="gqa_block_cached_fwd_bwd",
    )(x.reshape(rows), transposed(k_cache), transposed(v_cache), wq, wo, grad_out.reshape(rows))
    return (out.reshape(x.shape), dx.reshape(x.shape), restored(dk), restored(dv), dwq, dwo)
```

```python
import jax
import jax.numpy as jnp
from jax import lax
import jax.experimental.pallas as pl
import jax.experimental.pallas.tpu as pltpu

F32 = jnp.float32
BF16 = jnp.bfloat16
LOG2E = 1.4426950408889634

RING = 15
W_RING, DW_RING = 6, 5
BLOCK = 4
READ_CUTS = tuple((a, r, 8, a) for r in range(0, 96, 8) for a in (0, 1))
FIRST_CUTS = tuple((a, r, 24, a) for r in range(0, 384, 24) for a in (0, 1))
WRITE_CUTS = tuple((a, max(r, 0), min(r + 64, 384) - max(r, 0), a)
                   for r in range(24 - 64, 384, 64) for a in (0, 1))
POINTS = 5
READ_PHASES = ((2, 105), (230, 184), (425, 256))
SPARE_POINT, SPARE_STEPS = 1, (8, 20, 46, 48, 60, 85, 89, 98, 100)
WRITE_PHASES = ((25, 20), (65, 39), (102, 62))
EARLY_ROWS = 5


def _nn(a, b):
    return lax.dot_general(a, b, (((1,), (0,)), ((), ())), preferred_element_type=F32)


def _nt(a, b):
    return lax.dot_general(a, b, (((1,), (1,)), ((), ())), preferred_element_type=F32)


def _stack(parts):
    return jnp.concatenate(parts, axis=0).astype(BF16)


def _low_lanes(shape):
    return lax.broadcasted_iota(jnp.int32, shape, 1) < 64


def _scores(a, m_t):
    t = a[:, 128:256]
    low = _low_lanes(t.shape)
    first = _nn(a[:, 0:128].astype(BF16), m_t[0:128, :])
    mid = _nn(_stack([jnp.where(low, t, 0.0), jnp.where(low, 0.0, t)]), m_t[128:256, :])
    last = _nn(a[:, 256:384].astype(BF16), m_t[256:384, :])
    return first + mid[0:64], last + mid[64:128]


def _apply(w, m_t):
    first = _nt(w[0].astype(BF16), m_t[0:128, :])
    mid = _nt(_stack(w), m_t[128:256, :])
    last = _nt(w[1].astype(BF16), m_t[256:384, :])
    return jnp.concatenate(
        [first, jnp.where(_low_lanes(first.shape), mid[0:64], mid[64:128]), last], axis=1)


def _softmax(s):
    e = jnp.exp2((s - jnp.max(s, axis=1, keepdims=True)) * LOG2E)
    total = jnp.sum(e, axis=1, keepdims=True)
    return e * pltpu.reciprocal(total, approx=False, full_range=False)


def _softmax_grad(p, dp):
    return [a * (b - jnp.sum(a * b, axis=1, keepdims=True)) for a, b in zip(p, dp)]


def _cache_grad(a, w0, w1, dst):
    a_t = a.astype(BF16).T
    dh = a_t.shape[0] // 2
    for h in range(2):
        u = pltpu.bitcast(a_t[h * dh:(h + 1) * dh], jnp.uint32)
        low, zero = _low_lanes(u.shape), jnp.zeros_like(u)
        lhs = jnp.concatenate([pltpu.bitcast(jnp.where(low, u, zero), BF16),
                               pltpu.bitcast(jnp.where(low, zero, u), BF16)], axis=0)
        r = _nn(lhs, _stack([w0[h], w1[h]])).astype(BF16)
        dst[0, h * dh:(h + 1) * dh, :] = r[:dh]
        dst[1, h * dh:(h + 1) * dh, :] = r[dh:]


def _spread(a, b, run=2):
    keys = [((i // run + 0.5) / len(part), which, i)
            for which, part in enumerate((a, b)) for i in range(len(part))]
    return [(a, b)[which][i] for _, which, i in sorted(keys)]


def _mod(v, n):
    return v - n * lax.shift_right_logical(v * (65536 // n + 1), 16)


def _lookup(k, table):
    value = 0
    for key, v in table:
        value = jnp.where(k >= key, v, value)
    return value


@jax.jit
def pallas_standalone__gqa_block_cached__near_ridge_kernel(
    x: jax.Array,
    k_cache: jax.Array,
    v_cache: jax.Array,
    wq: jax.Array,
    wo: jax.Array,
    grad_out: jax.Array,
):
    nb, sq, d = x.shape
    _, nh, sk, dh = k_cache.shape
    assert (nb, sq, d, nh, dh) == (16, 64, 640, 32, 192) and wq.shape == (d, nh * dh)
    pw = 2 * dh
    n_pairs = nh // 2
    pair_steps = nb // 2
    n_steps = n_pairs * pair_steps
    n_units = n_steps // 2
    scale = dh ** -0.5
    spare_words = [(w, sum(1 << (s - w) for s in SPARE_STEPS if w <= s < w + 16))
                   for w in range(0, n_steps, 16)]

    def kernel(x_hbm, k_hbm, v_hbm, wq_hbm, wo_hbm, g_hbm,
               out_hbm, dx_hbm, dk_hbm, dv_hbm, dwq_hbm, dwo_hbm,
               x_v, g_v, wq_v, wo_v, k_v, v_v, dk_v, dv_v,
               out_acc, dx_acc, out_v, dx_v, dwq_acc, dwo_acc, dwq_v, dwo_v, sems):
        caches, cache_grads = ((k_hbm, k_v), (v_hbm, v_v)), ((dk_hbm, dk_v), (dv_hbm, dv_v))
        weights, weight_grads = (wq_hbm, wq_v, wo_hbm, wo_v), (dwq_hbm, dwq_v, dwo_hbm, dwo_v)
        inputs, outputs = ((x_hbm, x_v), (g_hbm, g_v)), ((out_hbm, out_v), (dx_hbm, dx_v))
        sem_weights, sem_first, sem_second, sem_last = (sems.at[2 * RING + i] for i in range(4))

        def weight_part(refs, p, slot, part, parts, pieces):
            q_hbm, q_v, o_hbm, o_v = refs
            a, b = d // parts, pw // parts
            q_rows = pl.ds(pl.multiple_of(part * a, 8), a)
            o_row = pl.multiple_of(part * b, 8)
            views = ((q_hbm.at[q_rows, pl.ds(pl.multiple_of(p * pw, pw), pw)],
                      q_v.at[slot, q_rows], a // pieces),
                     (o_hbm.at[pl.ds(pl.multiple_of(p * pw + o_row, 8), b), :],
                      o_v.at[slot, pl.ds(o_row, b)], b // pieces))
            return [(h.at[pl.ds(i * n, n)], v.at[pl.ds(i * n, n)], queue)
                    for i in range(pieces) for queue, (h, v, n) in enumerate(views)]

        def cache_part(refs, m, first, count, cuts, row0=0):
            p, batches = lax.shift_right_logical(m, 2), pl.ds(first, count)
            size = sum(cut[2] for cut in cuts) // 2
            in_unit = pl.ds(row0 if size == pw else pl.multiple_of(row0, 8), size)
            views = [(h.at[batches, m & 3, pl.ds(pl.multiple_of(p * pw + row0, 8), size), :],
                      v.at[_mod(m, RING), batches, in_unit, :]) for h, v in refs]
            return [(views[a][0].at[:, pl.ds(r, n), :], views[a][1].at[:, pl.ds(r, n), :], queue)
                    for a, r, n, queue in cuts]

        def row_part(refs, j, rows, starts):
            src = (pl.ds(2 * (j & 1), 2), lax.shift_right_logical(j, 1))
            return [(h.at[src + (pl.ds(r, rows),)], v.at[j, :, pl.ds(r, rows)], queue)
                    for r in starts for queue, (h, v) in enumerate(refs)]

        def outgoing(copies):
            return [(v, h, queue) for h, v, queue in copies]

        def read_group(c):
            m, p, e = lax.shift_right_logical(c, 2), lax.shift_right_logical(c, 4), c & 15
            nxt = jnp.minimum(p + 1, n_pairs - 1)
            rows = [pl.multiple_of((e & 1) * 32 + r, 16) for r in (0, 16)]
            return cache_part(caches, m, 0, 4, READ_CUTS, (c & 3) * (pw // 4)), [
                (p < n_pairs - 1, weight_part(weights, nxt, _mod(nxt, W_RING), e, 16, 1)),
                (p == 0, row_part(inputs, lax.shift_right_logical(e, 1), 16, rows))]

        def write_unit(m):
            p = lax.shift_right_logical(m, 2)
            src = jnp.minimum(p, n_pairs - 2)
            return (outgoing(cache_part(cache_grads, m, 0, 4, WRITE_CUTS)), p != n_pairs - 2,
                    outgoing(weight_part(weight_grads, src, _mod(src, DW_RING), m & 3, 4, 4)))

        def first_weights():
            return sum([weight_part(weights, 0, 0, u, 4, 4) for u in range(4)], [])

        def first_reads(j):
            return (row_part(inputs, j, 16, (0, 16, 32, 48))
                    + cache_part(caches, 0, 2 * j, 2, FIRST_CUTS)
                    + (weight_part(weights, 1, 1, 0, 4, 4) if j else []))

        def early_writes():
            return outgoing(sum([row_part(outputs, j, 32, (r,))
                                 for r in (0, 32) for j in range(EARLY_ROWS)], []))

        def last_writes(stage):
            p, m = n_pairs - 1, n_units - 1
            if stage == 0:
                rows = [row_part(outputs, j, 32, (0, 32)) for j in range(EARLY_ROWS, pair_steps - 1)]
                return outgoing(_spread(
                    cache_part(cache_grads, m, 0, 2, WRITE_CUTS),
                    sum(rows, []) + weight_part(weight_grads, p - 1, (p - 1) % DW_RING, 3, 4, 2)))
            cache = cache_part(cache_grads, m, 2, 2, WRITE_CUTS)
            rows = row_part(outputs, pair_steps - 1, 32, (0, 32))
            dw = sum([weight_part(weight_grads, p, p % DW_RING, u, 4, 2) for u in range(4)], [])
            if stage == 1:
                return outgoing(_spread(cache[1::2], _spread(dw[1::2], rows[0::2], 1), 1))
            return outgoing(_spread(cache[0::2], _spread(dw[0::2], rows[1::2], 1), 1))

        def start(copies, sem):
            for src, dst, queue in copies:
                pltpu.make_async_copy(src, dst, sem).start(priority=queue)

        def wait(copies, sem):
            for src, dst, _ in copies:
                pltpu.make_async_copy(src, dst, sem).wait()

        def wait_written(m):
            cache, has_dw, dw = write_unit(m)
            sem = sems.at[RING + _mod(m, RING)]
            wait(cache, sem)
            pl.when(has_dw)(lambda: wait(dw, sem))

        def acquire(m):
            cache, further = zip(*[read_group(4 * m + q) for q in range(4)])
            sem = sems.at[_mod(m, RING)]
            wait(sum(cache, []), sem)
            for n, (cond, _) in enumerate(further[0]):
                pl.when(cond)(lambda: wait(sum([more[n][1] for more in further], []), sem))
            pl.when(m >= RING)(lambda: wait_written(m - RING))

        def transfers(i, n_read, n_written, single):
            on = n_written < _lookup(i, WRITE_PHASES)
            cache, has_dw, dw = write_unit(n_written)
            sem, dw_on = sems.at[RING + _mod(n_written, RING)], on & has_dw
            todo = {"write": _spread([(on, c, sem) for c in cache], [(dw_on, c, sem) for c in dw]),
                    "more": []}
            n_written = n_written + jnp.where(on, 1, 0)
            for point in range(POINTS):
                on = n_read < _lookup(POINTS * i + point, READ_PHASES)
                if point == SPARE_POINT:
                    on = on & ((lax.shift_right_logical(_lookup(i, spare_words), i & 15) & 1) == 1)
                group = jnp.minimum(n_read, 4 * n_units - 1)
                cache, more = read_group(group)
                sem = sems.at[_mod(lax.shift_right_logical(group, 2), RING)]
                todo[point] = [(on, c, sem) for c in cache]
                for cond, copies in more if single else more[:1]:
                    both = on & cond
                    todo["more"] += [(both, c, sem) for c in copies]
                n_read = n_read + jnp.where(on, 1, 0)
            if single:
                todo["last"] = [(i == n_steps - 1, c, sem_last) for c in last_writes(1)]
            return todo, (n_read, n_written)

        def compute(i, send, may_begin, may_end):
            p, j, m = lax.shift_right_logical(i, 3), i & 7, lax.shift_right_logical(i, 1)
            at = (_mod(m, RING), pl.ds(2 * (i & 1), 2))
            k_t, v_t, dk_t, dv_t = k_v.at[at], v_v.at[at], dk_v.at[at], dv_v.at[at]
            wq_p, wo_p = wq_v.at[_mod(p, W_RING)], wo_v.at[_mod(p, W_RING)]

            def add_weight_grad(acc, staged, a, b):
                term = _nn(a.T, b)
                total = (jnp.where(j == 0, 0.0, acc[...]) if may_begin else acc[...]) + term
                acc[...] = total
                if may_end:
                    staged[_mod(p, DW_RING)] = total.astype(BF16)

            send(0)
            q = _nn(x_v[j].reshape(2 * sq, d), wq_p[...]) * scale
            s0 = _scores(q[:sq], k_t.at[0])
            send(1)
            do = _nt(g_v[j].reshape(2 * sq, d), wo_p[...])
            send("more")
            s1 = _scores(q[sq:], k_t.at[1])
            p0 = [_softmax(t) for t in s0]
            o0 = _apply(p0, v_t.at[0])
            dp0 = _scores(do[:sq], v_t.at[0])
            p1 = [_softmax(t) for t in s1]
            o1 = _apply(p1, v_t.at[1])
            send(2)
            _cache_grad(do, p0, p1, dv_t)
            dp1 = _scores(do[sq:], v_t.at[1])
            ds0 = _softmax_grad(p0, dp0)
            send("write")
            dq0 = _apply(ds0, k_t.at[0]) * scale
            ds1 = _softmax_grad(p1, dp1)
            o = _stack([o0, o1])
            add_weight_grad(dwo_acc, dwo_v, o, g_v[j].reshape(2 * sq, d))
            send(3)
            dq1 = _apply(ds1, k_t.at[1]) * scale
            send(4)
            total = out_acc[j] + _nn(o, wo_p[...])
            out_acc[j] = total
            out_v[j] = total.astype(BF16).reshape(2, sq, d)
            send("last")
            dq = _stack([dq0, dq1])
            add_weight_grad(dwq_acc, dwq_v, x_v[j].reshape(2 * sq, d), dq)
            total = dx_acc[j] + _nt(dq, wq_p[...])
            dx_acc[j] = total
            dx_v[j] = total.astype(BF16).reshape(2, sq, d)
            _cache_grad(q, ds0, ds1, dk_t)

        def step(i, counts, may_begin=True, may_end=True, single=True):
            todo, counts = transfers(i, *counts, single)

            def send(point):
                for n, (cond, copy, sem) in enumerate(todo.get(point, [])):
                    pl.when(cond & (i >= 0) if n & 2 else cond)(lambda: start([copy], sem))

            compute(i, send, may_begin, may_end)
            return counts

        def single_step(i, counts):
            pl.when(i == 1)(lambda: wait(first_reads(1), sem_second))
            pl.when((i > 1) & ((i & 1) == 0))(lambda: acquire(lax.shift_right_logical(i, 1)))
            pl.when(i == n_steps - 3)(lambda: start(early_writes(), sem_last))

            @pl.when(i == n_steps - 2)
            def _():
                cache, _, dw = write_unit(n_units - 2)
                start(_spread(cache, dw), sems.at[RING + (n_units - 2) % RING])

            pl.when(i == n_steps - 1)(lambda: start(last_writes(0), sem_last))
            return step(i, counts)

        def block(b, counts):
            i = BLOCK * (b + 1)
            for u in range(0, BLOCK, 2):
                acquire(lax.shift_right_logical(i + u, 1))
            for u in range(BLOCK):
                counts = step(i + u, counts, u == 0, u == BLOCK - 1, False)
            return counts

        def half(h, counts):
            begin = h * (n_steps - BLOCK)
            counts = lax.fori_loop(begin, begin + BLOCK, single_step, counts)
            return lax.fori_loop(0, (1 - h) * (n_steps // BLOCK - 2), block, counts)

        def zero(acc, part, parts):
            n = acc.shape[0] // parts
            acc[pl.ds(pl.multiple_of(part * n, 8), n), :] = jnp.zeros((n, acc.shape[1]), F32)

        start(first_weights(), sem_weights)
        start(first_reads(0), sem_first)

        @pl.loop(0, 16)
        def _(n):
            zero(dwq_acc, n, 16)
            zero(dwo_acc, n, 16)

        @pl.loop(0, 8 * pair_steps)
        def _(n):
            zero(out_acc.at[lax.shift_right_logical(n, 3)], n & 7, 8)
            zero(dx_acc.at[lax.shift_right_logical(n, 3)], n & 7, 8)

        wait(first_weights(), sem_weights)
        start(first_reads(1)[:12], sem_second)
        wait(first_reads(0), sem_first)
        start(first_reads(1)[12:], sem_second)
        lax.fori_loop(0, 2, half, (4, 0))
        start(last_writes(2), sem_last)
        pl.loop(n_units - RING, n_units - 1)(wait_written)
        wait(early_writes() + sum([last_writes(stage) for stage in range(3)], []), sem_last)

    def transposed(c):
        return jnp.swapaxes(c, 2, 3).reshape(4, nb // 4, nh * dh, sk)

    def restored(c):
        return jnp.swapaxes(c.reshape(nb, nh, dh, sk), 2, 3)

    rows, staged, summed = (4, nb // 4, sq, d), (pair_steps, 2, sq, d), (pair_steps, 2 * sq, d)
    hbm = pl.BlockSpec(memory_space=pl.ANY)
    vmem = pltpu.VMEM
    out, dx, dk, dv, dwq, dwo = pl.pallas_call(
        kernel,
        in_specs=[hbm] * 6,
        out_specs=[hbm] * 6,
        out_shape=[
            jax.ShapeDtypeStruct(rows, x.dtype),
            jax.ShapeDtypeStruct(rows, x.dtype),
            jax.ShapeDtypeStruct((4, nb // 4, nh * dh, sk), k_cache.dtype),
            jax.ShapeDtypeStruct((4, nb // 4, nh * dh, sk), v_cache.dtype),
            jax.ShapeDtypeStruct(wq.shape, wq.dtype),
            jax.ShapeDtypeStruct(wo.shape, wo.dtype),
        ],
        scratch_shapes=[
            vmem(staged, BF16), vmem(staged, BF16),
            vmem((W_RING, d, pw), BF16), vmem((W_RING, pw, d), BF16),
            vmem((RING, 4, pw, sk), BF16), vmem((RING, 4, pw, sk), BF16),
            vmem((RING, 4, pw, sk), BF16), vmem((RING, 4, pw, sk), BF16),
            vmem(summed, F32), vmem(summed, F32), vmem(staged, BF16), vmem(staged, BF16),
            vmem((d, pw), F32), vmem((pw, d), F32),
            vmem((DW_RING, d, pw), BF16), vmem((DW_RING, pw, d), BF16),
            pltpu.SemaphoreType.DMA((2 * RING + 4,)),
        ],
        compiler_params=pltpu.CompilerParams(
            vmem_limit_bytes=120 * 1024 * 1024, disable_bounds_checks=True),
        name="gqa_block_cached_fwd_bwd",
    )(x.reshape(rows), transposed(k_cache), transposed(v_cache), wq, wo, grad_out.reshape(rows))
    return (out.reshape(x.shape), dx.reshape(x.shape), restored(dk), restored(dv), dwq, dwo)
```
